```python
import os as _os
_os.environ.setdefault("JAX_PLATFORMS", "cpu")
import jax
import jax.numpy as jnp

def _softmax(x, axis=-1):
    return jax.nn.softmax(x, axis=axis)
def _gelu(x):
    return jax.nn.gelu(x, approximate=True)
def _silu(x):
    return jax.nn.silu(x)
def _sigmoid(x):
    return jax.nn.sigmoid(x)
def _layernorm(x, axis=-1, eps=1e-5):
    m = jnp.mean(x, axis=axis, keepdims=True)
    v = jnp.var(x, axis=axis, keepdims=True)
    return (x - m) / jnp.sqrt(v + eps)
def _scatter_add(tgt, idx, src, axis=0):
    return tgt.at[idx].add(src)
def _segment_sum(src, seg, n):
    return jax.ops.segment_sum(src, seg, n)
class _Rng:
    def __init__(self, key):
        self._k = key
    def _next(self):
        self._k, sub = jax.random.split(self._k)
        return sub
    def normal(self, shape):
        return jax.random.normal(self._next(), shape, dtype=jnp.bfloat16)
    def randint(self, lo, hi, shape):
        return jax.random.randint(self._next(), shape, lo, hi, dtype=jnp.int32)
    def uniform(self, shape, lo=0.0, hi=1.0):
        return jax.random.uniform(self._next(), shape, jnp.bfloat16, lo, hi)
    def permutation(self, n):
        return jax.random.permutation(self._next(), n)


kernel_name = 'gated_mix__mha_block__mha_block__prompt'

def setup_inputs():
    _rng = _Rng(jax.random.key(int.from_bytes(__import__("os").urandom(4), "little")))
    _w = (lambda a: (lambda t: t.astype(jnp.bfloat16) if jnp.issubdtype(t.dtype, jnp.floating) else t)(jnp.asarray(a)))
    def _A_setup():
        B, S, D, H = 1, 2048, 448, 16
        return {
            "x": _w((lambda *s: _rng.normal(s) * 0.05)(B, S, D)),
            "wqkv": _w((lambda *s: _rng.normal(s) * 0.4)(D, 3 * D)),
            "wo": _w((lambda *s: _rng.normal(s) * 0.05)(D, D)),
        }
    _A_in = _A_setup()

    def _B_setup():
        B, S, D, H = 1, 2048, 448, 16
        return {
            "x": _w((lambda *s: _rng.normal(s) * 0.05)(B, S, D)),
            "wqkv": _w((lambda *s: _rng.normal(s) * 0.4)(D, 3 * D)),
            "wo": _w((lambda *s: _rng.normal(s) * 0.05)(D, D)),
        }
    _B_in = _B_setup()

    return {
        "A_x": _A_in["x"],
        "A_wqkv": _A_in["wqkv"],
        "A_wo": _A_in["wo"],
        "B_x": _B_in["x"],
        "B_wqkv": _B_in["wqkv"],
        "B_wo": _B_in["wo"],
        "gate_w": _w((lambda *s: _rng.normal(s) * 0.05)(448) * 16.0),
    }

def reference(A_x, A_wqkv, A_wo, B_x, B_wqkv, B_wo, gate_w):
    def _A_ref(x, wqkv, wo):
        B, S, D = x.shape
        H = 16
        Dh = D // H
        qkv = (lambda x, *d: x.transpose(*d))((x @ wqkv).reshape(B, S, 3, H, Dh), 2, 0, 3, 1, 4)
        q, k, v = qkv[0], qkv[1], qkv[2]
        scores = jnp.einsum("bhqd,bhkd->bhqk", q, k) * (Dh ** -0.5)
        p = _softmax(scores, axis=-1)
        o = jnp.einsum("bhqk,bhkd->bhqd", p, v)
        return (lambda x, *d: x.transpose(*d))(o, 0, 2, 1, 3).reshape(B, S, D) @ wo

    def _B_ref(x, wqkv, wo):
        B, S, D = x.shape
        H = 16
        Dh = D // H
        qkv = (lambda x, *d: x.transpose(*d))((x @ wqkv).reshape(B, S, 3, H, Dh), 2, 0, 3, 1, 4)
        q, k, v = qkv[0], qkv[1], qkv[2]
        scores = jnp.einsum("bhqd,bhkd->bhqk", q, k) * (Dh ** -0.5)
        p = _softmax(scores, axis=-1)
        o = jnp.einsum("bhqk,bhkd->bhqd", p, v)
        return (lambda x, *d: x.transpose(*d))(o, 0, 2, 1, 3).reshape(B, S, D) @ wo

    x = A_x
    g = _sigmoid((x * gate_w).sum(-1, keepdims=True))
    a = _A_ref(x, A_wqkv, A_wo)
    b = _B_ref(x, B_wqkv, B_wo)
    return g * a + (1 - g) * b
```

```python
import functools
import math

import jax
import jax.numpy as jnp
import jax.experimental.pallas as pl
import jax.experimental.pallas.tpu as pltpu

S = 2048
D = 448
H = 16
DH = 28
DP = 32
HP = H * DP
NB = 2
NH = NB * H
NG = NH // 4
TQ = 512
NQ = S // TQ
NIT = NH * NQ
GR = 16

_QSCALE = (DH ** -0.5) * math.log2(math.e)


def _kernel(x_ref, wk_ref, wqv_ref, wo_ref, o_ref,
            k_scr, qt_scr, vt_scr, g_scr, s0_scr, s1_scr, ot_scr):
    f32 = jnp.float32
    bf16 = jnp.bfloat16

    for rb in range(S // 512):
        xr = x_ref[rb * 512:(rb + 1) * 512, :]
        kk = jnp.dot(xr, wk_ref[...], preferred_element_type=f32)
        for g in range(NG):
            k_scr[g, rb * 512:(rb + 1) * 512, :] = kk[:, g * 128:(g + 1) * 128].astype(bf16)

    row = jax.lax.broadcasted_iota(jnp.int32, (HP, TQ), 0)
    ones_row = (row % DP) == DH
    for qb in range(NQ):
        xr = x_ref[qb * TQ:(qb + 1) * TQ, :]
        for br in range(NB):
            base = br * 2 * HP
            qt = jax.lax.dot_general(wqv_ref[base:base + HP, :], xr,
                                     (((1,), (1,)), ((), ())),
                                     preferred_element_type=f32)
            qt = (qt * _QSCALE).astype(bf16)
            for gg in range(4):
                qt_scr[br * 4 + gg, qb] = qt[gg * 128:(gg + 1) * 128, :]
            vt = jax.lax.dot_general(wqv_ref[base + HP:base + 2 * HP, :], xr,
                                     (((1,), (1,)), ((), ())),
                                     preferred_element_type=f32)
            vt = jnp.where(ones_row, 1.0, vt).astype(bf16)
            for h in range(H):
                vt_scr[br * H + h, :, qb * TQ:(qb + 1) * TQ] = vt[h * DP:(h + 1) * DP, :]
        gl = jax.lax.dot_general(wqv_ref[2 * NB * HP:2 * NB * HP + GR, :], xr,
                                 (((1,), (1,)), ((), ())),
                                 preferred_element_type=f32)
        gate = jax.nn.sigmoid(gl[0:8, :])
        g_scr[0, qb] = gate
        g_scr[1, qb] = 1.0 - gate

    qrow = jax.lax.broadcasted_iota(jnp.int32, (128, TQ), 0) // DP

    def qk(it, s_scr):
        hh = it // NQ
        qb = it % NQ
        g = hh // 4
        j = hh % 4
        qt = qt_scr[g, qb]
        qm = jnp.where(qrow == j, qt, jnp.zeros_like(qt))
        s = jnp.dot(k_scr[g], qm, preferred_element_type=f32)
        s_scr[...] = s
        return jnp.max(s, axis=0, keepdims=True)

    def pv(it, s_scr, m):
        hh = it // NQ
        qb = it % NQ
        p = jnp.exp2(s_scr[...] - m).astype(bf16)
        o = jnp.dot(vt_scr[hh], p, preferred_element_type=f32)
        l = o[DH:DH + 1, :]
        gf = g_scr[hh // H, qb][0:1, :]
        r0 = pl.multiple_of(hh * DP, DP)
        ot_scr[qb, pl.ds(r0, DP), :] = (o * (gf / l)).astype(bf16)

    m0 = qk(0, s0_scr)

    def body(i, m_a):
        it = 2 * i
        m_b = qk(it + 1, s1_scr)
        pv(it, s0_scr, m_a)
        m_a2 = qk(jnp.minimum(it + 2, NIT - 1), s0_scr)
        pv(it + 1, s1_scr, m_b)
        return m_a2

    jax.lax.fori_loop(0, NIT // 2, body, m0)

    for qb in range(NQ):
        ot = jnp.dot(wo_ref[...], ot_scr[qb], preferred_element_type=f32)
        o_ref[qb * TQ:(qb + 1) * TQ, :] = ot.T.astype(o_ref.dtype)


def _pad_heads(w):
    w = w.reshape(D, 3, H, DH)
    w = jnp.pad(w, ((0, 0), (0, 0), (0, 0), (0, DP - DH)))
    return w.reshape(D, 3, HP)


def _pad_wo(wo):
    wo = wo.reshape(H, DH, D)
    wo = jnp.pad(wo, ((0, 0), (0, DP - DH), (0, 0)))
    return wo.reshape(HP, D)


@jax.jit
def pallas_gated_mix__mha_block__mha_block__prompt_kernel(
    A_x: jax.Array,
    A_wqkv: jax.Array,
    A_wo: jax.Array,
    B_x: jax.Array,
    B_wqkv: jax.Array,
    B_wo: jax.Array,
    gate_w: jax.Array,
):
    x = A_x.reshape(S, D)
    wa = _pad_heads(A_wqkv)
    wb = _pad_heads(B_wqkv)
    wk = jnp.concatenate([wa[:, 1, :], wb[:, 1, :]], axis=1)
    gw = jnp.pad(gate_w.reshape(1, D), ((0, GR - 1), (0, 0)))
    wqv = jnp.concatenate([wa[:, 0, :].T, wa[:, 2, :].T,
                           wb[:, 0, :].T, wb[:, 2, :].T, gw], axis=0)
    wo = jnp.concatenate([_pad_wo(A_wo), _pad_wo(B_wo)], axis=0).T

    out = pl.pallas_call(
        _kernel,
        out_shape=jax.ShapeDtypeStruct((S, D), jnp.bfloat16),
        scratch_shapes=[
            pltpu.VMEM((NG, S, 128), jnp.bfloat16),
            pltpu.VMEM((NG, NQ, 128, TQ), jnp.bfloat16),
            pltpu.VMEM((NH, DP, S), jnp.bfloat16),
            pltpu.VMEM((NB, NQ, 8, TQ), jnp.float32),
            pltpu.VMEM((S, TQ), jnp.float32),
            pltpu.VMEM((S, TQ), jnp.float32),
            pltpu.VMEM((NQ, NH * DP, TQ), jnp.bfloat16),
        ],
        compiler_params=pltpu.CompilerParams(vmem_limit_bytes=100 * 1024 * 1024),
    )(x, wk, wqv, wo)
    return out.reshape(1, S, D)
```

```python
import functools
import math

import jax
import jax.numpy as jnp
import jax.experimental.pallas as pl
import jax.experimental.pallas.tpu as pltpu

S = 2048
D = 448
H = 16
DH = 28
DP = 32
HP = H * DP
NB = 2
NH = NB * H
NG = NH // 4
TQ = 512
NQ = S // TQ
NIT = NH * NQ
GR = 16
CK = 256

_QSCALE = (DH ** -0.5) * math.log2(math.e)


def _kernel(x_ref, wk_ref, wqv_ref, wo_ref, o_ref,
            k_scr, qt_scr, vt_scr, g_scr, s0_scr, s1_scr, ot_scr):
    f32 = jnp.float32
    bf16 = jnp.bfloat16

    for rb in range(S // 512):
        xr = x_ref[rb * 512:(rb + 1) * 512, :]
        kk = jnp.dot(xr, wk_ref[...], preferred_element_type=f32)
        for g in range(NG):
            k_scr[g, rb * 512:(rb + 1) * 512, :] = kk[:, g * 128:(g + 1) * 128].astype(bf16)

    row = jax.lax.broadcasted_iota(jnp.int32, (HP, TQ), 0)
    ones_row = (row % DP) == DH
    for qb in range(NQ):
        xr = x_ref[qb * TQ:(qb + 1) * TQ, :]
        for br in range(NB):
            base = br * 2 * HP
            qt = jax.lax.dot_general(wqv_ref[base:base + HP, :], xr,
                                     (((1,), (1,)), ((), ())),
                                     preferred_element_type=f32)
            qt = (qt * _QSCALE).astype(bf16)
            for gg in range(4):
                qt_scr[br * 4 + gg, qb] = qt[gg * 128:(gg + 1) * 128, :]
            vt = jax.lax.dot_general(wqv_ref[base + HP:base + 2 * HP, :], xr,
                                     (((1,), (1,)), ((), ())),
                                     preferred_element_type=f32)
            vt = jnp.where(ones_row, 1.0, vt).astype(bf16)
            for h in range(H):
                vt_scr[br * H + h, :, qb * TQ:(qb + 1) * TQ] = vt[h * DP:(h + 1) * DP, :]
        gl = jax.lax.dot_general(wqv_ref[2 * NB * HP:2 * NB * HP + GR, :], xr,
                                 (((1,), (1,)), ((), ())),
                                 preferred_element_type=f32)
        gate = jax.nn.sigmoid(gl[0:8, :])
        g_scr[0, qb] = gate
        g_scr[1, qb] = 1.0 - gate

    qrow = jax.lax.broadcasted_iota(jnp.int32, (128, TQ), 0) // DP

    def qm_of(it):
        hh = it // NQ
        qb = it % NQ
        qt = qt_scr[hh // 4, qb]
        return jnp.where(qrow == hh % 4, qt, jnp.zeros_like(qt))

    def step(it_n, s_n, it_c, s_c, m_c):
        g = (it_n // NQ) // 4
        qm = qm_of(it_n)
        hh = it_c // NQ
        qb = it_c % NQ
        m8 = None
        acc = None
        for c in range(S // CK):
            rows = slice(c * CK, (c + 1) * CK)
            s = jnp.dot(k_scr[g, rows, :], qm, preferred_element_type=f32)
            s_n[rows, :] = s
            mc = jnp.max(s.reshape(CK // 8, 8, TQ), axis=0)
            m8 = mc if m8 is None else jnp.maximum(m8, mc)
            p = jnp.exp2(s_c[rows, :] - m_c).astype(bf16)
            o = jnp.dot(vt_scr[hh, :, rows], p, preferred_element_type=f32)
            acc = o if acc is None else acc + o
        l = acc[DH:DH + 1, :]
        gf = g_scr[hh // H, qb][0:1, :]
        r0 = pl.multiple_of(hh * DP, DP)
        ot_scr[qb, pl.ds(r0, DP), :] = (acc * (gf / l)).astype(bf16)
        return jnp.max(m8, axis=0, keepdims=True)

    s = jnp.dot(k_scr[0], qm_of(0), preferred_element_type=f32)
    s0_scr[...] = s
    m0 = jnp.max(s, axis=0, keepdims=True)

    def body(i, m_a):
        it = 2 * i
        m_b = step(it + 1, s1_scr, it, s0_scr, m_a)
        m_a2 = step(jnp.minimum(it + 2, NIT - 1), s0_scr, it + 1, s1_scr, m_b)
        return m_a2

    jax.lax.fori_loop(0, NIT // 2, body, m0)

    for qb in range(NQ):
        ot = jnp.dot(wo_ref[...], ot_scr[qb], preferred_element_type=f32)
        o_ref[qb * TQ:(qb + 1) * TQ, :] = ot.T.astype(o_ref.dtype)


def _pad_heads(w):
    w = w.reshape(D, 3, H, DH)
    w = jnp.pad(w, ((0, 0), (0, 0), (0, 0), (0, DP - DH)))
    return w.reshape(D, 3, HP)


def _pad_wo(wo):
    wo = wo.reshape(H, DH, D)
    wo = jnp.pad(wo, ((0, 0), (0, DP - DH), (0, 0)))
    return wo.reshape(HP, D)


@jax.jit
def pallas_gated_mix__mha_block__mha_block__prompt_kernel(
    A_x: jax.Array,
    A_wqkv: jax.Array,
    A_wo: jax.Array,
    B_x: jax.Array,
    B_wqkv: jax.Array,
    B_wo: jax.Array,
    gate_w: jax.Array,
):
    x = A_x.reshape(S, D)
    wa = _pad_heads(A_wqkv)
    wb = _pad_heads(B_wqkv)
    wk = jnp.concatenate([wa[:, 1, :], wb[:, 1, :]], axis=1)
    gw = jnp.pad(gate_w.reshape(1, D), ((0, GR - 1), (0, 0)))
    wqv = jnp.concatenate([wa[:, 0, :].T, wa[:, 2, :].T,
                           wb[:, 0, :].T, wb[:, 2, :].T, gw], axis=0)
    wo = jnp.concatenate([_pad_wo(A_wo), _pad_wo(B_wo)], axis=0).T

    out = pl.pallas_call(
        _kernel,
        out_shape=jax.ShapeDtypeStruct((S, D), jnp.bfloat16),
        scratch_shapes=[
            pltpu.VMEM((NG, S, 128), jnp.bfloat16),
            pltpu.VMEM((NG, NQ, 128, TQ), jnp.bfloat16),
            pltpu.VMEM((NH, DP, S), jnp.bfloat16),
            pltpu.VMEM((NB, NQ, 8, TQ), jnp.float32),
            pltpu.VMEM((S, TQ), jnp.float32),
            pltpu.VMEM((S, TQ), jnp.float32),
            pltpu.VMEM((NQ, NH * DP, TQ), jnp.bfloat16),
        ],
        compiler_params=pltpu.CompilerParams(vmem_limit_bytes=100 * 1024 * 1024),
    )(x, wk, wqv, wo)
    return out.reshape(1, S, D)
```

```python
import functools
import math

import jax
import jax.numpy as jnp
import jax.experimental.pallas as pl
import jax.experimental.pallas.tpu as pltpu

S = 2048
D = 448
H = 16
DH = 28
DP = 32
HP = H * DP
NB = 2
NH = NB * H
NG = NH // 4
TQ = 512
NQ = S // TQ
NIT = NH * NQ
GR = 16
CK = 256

_QSCALE = (DH ** -0.5) * math.log2(math.e)


def _kernel(x_ref, wk_ref, wqv_ref, wo_ref, o_ref,
            k_scr, qt_scr, vt_scr, g_scr, s0_scr, ot_scr):
    f32 = jnp.float32
    bf16 = jnp.bfloat16

    for rb in range(S // 512):
        xr = x_ref[rb * 512:(rb + 1) * 512, :]
        kk = jnp.dot(xr, wk_ref[...], preferred_element_type=f32)
        for g in range(NG):
            k_scr[g, rb * 512:(rb + 1) * 512, :] = kk[:, g * 128:(g + 1) * 128].astype(bf16)

    row = jax.lax.broadcasted_iota(jnp.int32, (HP, TQ), 0)
    ones_row = (row % DP) == DH
    for qb in range(NQ):
        xr = x_ref[qb * TQ:(qb + 1) * TQ, :]
        for br in range(NB):
            base = br * 2 * HP
            qt = jax.lax.dot_general(wqv_ref[base:base + HP, :], xr,
                                     (((1,), (1,)), ((), ())),
                                     preferred_element_type=f32)
            qt = (qt * _QSCALE).astype(bf16)
            for gg in range(4):
                qt_scr[br * 4 + gg, qb] = qt[gg * 128:(gg + 1) * 128, :]
            vt = jax.lax.dot_general(wqv_ref[base + HP:base + 2 * HP, :], xr,
                                     (((1,), (1,)), ((), ())),
                                     preferred_element_type=f32)
            vt = jnp.where(ones_row, 1.0, vt).astype(bf16)
            for h in range(H):
                vt_scr[br * H + h, :, qb * TQ:(qb + 1) * TQ] = vt[h * DP:(h + 1) * DP, :]
        gl = jax.lax.dot_general(wqv_ref[2 * NB * HP:2 * NB * HP + GR, :], xr,
                                 (((1,), (1,)), ((), ())),
                                 preferred_element_type=f32)
        gate = jax.nn.sigmoid(gl[0:8, :])
        g_scr[0, qb] = gate
        g_scr[1, qb] = 1.0 - gate

    qrow = jax.lax.broadcasted_iota(jnp.int32, (128, TQ), 0) // DP

    def qm_of(it):
        hh = it // NQ
        qb = it % NQ
        qt = qt_scr[hh // 4, qb]
        return jnp.where(qrow == hh % 4, qt, jnp.zeros_like(qt))

    def body(it_c, m_c):
        it_n = jnp.minimum(it_c + 1, NIT - 1)
        g = (it_n // NQ) // 4
        qm = qm_of(it_n)
        hh = it_c // NQ
        qb = it_c % NQ
        m8 = None
        acc = None
        for c in range(S // CK):
            rows = slice(c * CK, (c + 1) * CK)
            s = jnp.dot(k_scr[g, rows, :], qm, preferred_element_type=f32)
            p = jnp.exp2(s0_scr[rows, :] - m_c).astype(bf16)
            s0_scr[rows, :] = s
            mc = jnp.max(s.reshape(CK // 8, 8, TQ), axis=0)
            m8 = mc if m8 is None else jnp.maximum(m8, mc)
            o = jnp.dot(vt_scr[hh, :, rows], p, preferred_element_type=f32)
            acc = o if acc is None else acc + o
        l = acc[DH:DH + 1, :]
        gf = g_scr[hh // H, qb][0:1, :]
        r0 = pl.multiple_of(hh * DP, DP)
        ot_scr[qb, pl.ds(r0, DP), :] = (acc * (gf / l)).astype(bf16)
        return jnp.max(m8, axis=0, keepdims=True)

    s = jnp.dot(k_scr[0], qm_of(0), preferred_element_type=f32)
    s0_scr[...] = s
    m0 = jnp.max(s, axis=0, keepdims=True)
    jax.lax.fori_loop(0, NIT, body, m0)

    for qb in range(NQ):
        ot = jnp.dot(wo_ref[...], ot_scr[qb], preferred_element_type=f32)
        o_ref[qb * TQ:(qb + 1) * TQ, :] = ot.T.astype(o_ref.dtype)


def _pad_heads(w):
    w = w.reshape(D, 3, H, DH)
    w = jnp.pad(w, ((0, 0), (0, 0), (0, 0), (0, DP - DH)))
    return w.reshape(D, 3, HP)


def _pad_wo(wo):
    wo = wo.reshape(H, DH, D)
    wo = jnp.pad(wo, ((0, 0), (0, DP - DH), (0, 0)))
    return wo.reshape(HP, D)


@jax.jit
def pallas_gated_mix__mha_block__mha_block__prompt_kernel(
    A_x: jax.Array,
    A_wqkv: jax.Array,
    A_wo: jax.Array,
    B_x: jax.Array,
    B_wqkv: jax.Array,
    B_wo: jax.Array,
    gate_w: jax.Array,
):
    x = A_x.reshape(S, D)
    wa = _pad_heads(A_wqkv)
    wb = _pad_heads(B_wqkv)
    wk = jnp.concatenate([wa[:, 1, :], wb[:, 1, :]], axis=1)
    gw = jnp.pad(gate_w.reshape(1, D), ((0, GR - 1), (0, 0)))
    wqv = jnp.concatenate([wa[:, 0, :].T, wa[:, 2, :].T,
                           wb[:, 0, :].T, wb[:, 2, :].T, gw], axis=0)
    wo = jnp.concatenate([_pad_wo(A_wo), _pad_wo(B_wo)], axis=0).T

    out = pl.pallas_call(
        _kernel,
        out_shape=jax.ShapeDtypeStruct((S, D), jnp.bfloat16),
        scratch_shapes=[
            pltpu.VMEM((NG, S, 128), jnp.bfloat16),
            pltpu.VMEM((NG, NQ, 128, TQ), jnp.bfloat16),
            pltpu.VMEM((NH, DP, S), jnp.bfloat16),
            pltpu.VMEM((NB, NQ, 8, TQ), jnp.float32),
            pltpu.VMEM((S, TQ), jnp.float32),
            pltpu.VMEM((NQ, NH * DP, TQ), jnp.bfloat16),
        ],
        compiler_params=pltpu.CompilerParams(vmem_limit_bytes=100 * 1024 * 1024),
    )(x, wk, wqv, wo)
    return out.reshape(1, S, D)
```

```python
import math

import jax
import jax.numpy as jnp
import jax.experimental.pallas as pl
import jax.experimental.pallas.tpu as pltpu

S = 2048
D = 448
H = 16
DH = 28
DP = 32
HP = H * DP
NB = 2
NH = NB * H
NG = NH // 4
TQ = 512
NQ = S // TQ
GR = 16
CK = 256

_QSCALE = (DH ** -0.5) * math.log2(math.e)
_NT = (((1,), (1,)), ((), ()))


def _kernel(x_ref, wa_ref, wb_ref, woa_ref, wob_ref, gw_ref, o_ref,
            wt_scr, wot_scr, k_scr, qt_scr, vt_scr, g_scr, s_scr, ot_scr):
    f32 = jnp.float32
    bf16 = jnp.bfloat16
    w_refs = (wa_ref, wb_ref)
    wo_refs = (woa_ref, wob_ref)

    for br in range(NB):
        wt_scr[2 * br] = w_refs[br][:, 0:HP].T
        wt_scr[2 * br + 1] = w_refs[br][:, 2 * HP:3 * HP].T
        wot_scr[:, br * HP:(br + 1) * HP] = wo_refs[br][...].T

    for rb in range(S // 512):
        xr = x_ref[rb * 512:(rb + 1) * 512, :]
        for br in range(NB):
            kk = jnp.dot(xr, w_refs[br][:, HP:2 * HP], preferred_element_type=f32)
            for gg in range(4):
                k_scr[br * 4 + gg, rb * 512:(rb + 1) * 512, :] = (
                    kk[:, gg * 128:(gg + 1) * 128].astype(bf16))

    row = jax.lax.broadcasted_iota(jnp.int32, (HP, TQ), 0)
    ones_row = (row % DP) == DH
    gw = jnp.broadcast_to(gw_ref[...], (GR, D))
    for qb in range(NQ):
        xr = x_ref[qb * TQ:(qb + 1) * TQ, :]
        for br in range(NB):
            qt = jax.lax.dot_general(wt_scr[2 * br], xr, _NT, preferred_element_type=f32)
            qt = (qt * _QSCALE).astype(bf16)
            for gg in range(4):
                qt_scr[br * 4 + gg, qb] = qt[gg * 128:(gg + 1) * 128, :]
            vt = jax.lax.dot_general(wt_scr[2 * br + 1], xr, _NT, preferred_element_type=f32)
            vt = jnp.where(ones_row, 1.0, vt).astype(bf16)
            for h in range(H):
                vt_scr[br * H + h, :, qb * TQ:(qb + 1) * TQ] = vt[h * DP:(h + 1) * DP, :]
        gl = jax.lax.dot_general(gw, xr, _NT, preferred_element_type=f32)
        gate = jax.nn.sigmoid(gl[0:8, :])
        g_scr[0, qb] = gate
        g_scr[1, qb] = 1.0 - gate

    qrow = jax.lax.broadcasted_iota(jnp.int32, (128, TQ), 0) // DP

    def qm_of(hh, qb):
        qt = qt_scr[hh // 4, qb]
        return jnp.where(qrow == hh % 4, qt, jnp.zeros_like(qt))

    def head_step(hh, ms, do_qk):
        hn = hh + 1
        g = hn // 4
        r0 = pl.multiple_of(hh * DP, DP)
        out_ms = []
        for qb in range(NQ):
            if do_qk:
                qm = qm_of(hn, qb)
            m_c = ms[qb]
            m8 = None
            acc = None
            for c in range(S // CK):
                rows = slice(c * CK, (c + 1) * CK)
                if do_qk:
                    s = jnp.dot(k_scr[g, rows, :], qm, preferred_element_type=f32)
                p = jnp.exp2(s_scr[qb, rows, :] - m_c).astype(bf16)
                if do_qk:
                    s_scr[qb, rows, :] = s
                    mc = jnp.max(s.reshape(CK // 8, 8, TQ), axis=0)
                    m8 = mc if m8 is None else jnp.maximum(m8, mc)
                o = jnp.dot(vt_scr[hh, :, rows], p, preferred_element_type=f32)
                acc = o if acc is None else acc + o
            l = acc[DH:DH + 1, :]
            gf = g_scr[hh // H, qb][0:1, :]
            ot_scr[qb, pl.ds(r0, DP), :] = (acc * (gf / l)).astype(bf16)
            if do_qk:
                out_ms.append(jnp.max(m8, axis=0, keepdims=True))
        return tuple(out_ms)

    ms0 = []
    for qb in range(NQ):
        s = jnp.dot(k_scr[0], qm_of(0, qb), preferred_element_type=f32)
        s_scr[qb] = s
        ms0.append(jnp.max(s, axis=0, keepdims=True))
    ms = jax.lax.fori_loop(0, NH - 1, lambda hh, ms: head_step(hh, ms, True), tuple(ms0))
    head_step(NH - 1, ms, False)

    for qb in range(NQ):
        ot = jnp.dot(wot_scr[...], ot_scr[qb], preferred_element_type=f32)
        o_ref[qb * TQ:(qb + 1) * TQ, :] = ot.T.astype(o_ref.dtype)


def _pad_heads(w):
    w = w.reshape(D, 3 * H, DH)
    w = jnp.pad(w, ((0, 0), (0, 0), (0, DP - DH)))
    return w.reshape(D, 3 * HP)


def _pad_wo(wo):
    wo = wo.reshape(H, DH, D)
    wo = jnp.pad(wo, ((0, 0), (0, DP - DH), (0, 0)))
    return wo.reshape(HP, D)


@jax.jit
def pallas_gated_mix__mha_block__mha_block__prompt_kernel(
    A_x: jax.Array,
    A_wqkv: jax.Array,
    A_wo: jax.Array,
    B_x: jax.Array,
    B_wqkv: jax.Array,
    B_wo: jax.Array,
    gate_w: jax.Array,
):
    x = A_x.reshape(S, D)
    out = pl.pallas_call(
        _kernel,
        out_shape=jax.ShapeDtypeStruct((S, D), jnp.bfloat16),
        scratch_shapes=[
            pltpu.VMEM((2 * NB, HP, D), jnp.bfloat16),
            pltpu.VMEM((D, NB * HP), jnp.bfloat16),
            pltpu.VMEM((NG, S, 128), jnp.bfloat16),
            pltpu.VMEM((NG, NQ, 128, TQ), jnp.bfloat16),
            pltpu.VMEM((NH, DP, S), jnp.bfloat16),
            pltpu.VMEM((NB, NQ, 8, TQ), jnp.float32),
            pltpu.VMEM((NQ, S, TQ), jnp.float32),
            pltpu.VMEM((NQ, NH * DP, TQ), jnp.bfloat16),
        ],
        compiler_params=pltpu.CompilerParams(vmem_limit_bytes=100 * 1024 * 1024),
    )(x, _pad_heads(A_wqkv), _pad_heads(B_wqkv), _pad_wo(A_wo), _pad_wo(B_wo),
      gate_w.reshape(1, D))
    return out.reshape(1, S, D)
```

```python
import math

import jax
import jax.numpy as jnp
import jax.experimental.pallas as pl
import jax.experimental.pallas.tpu as pltpu

S = 2048
D = 448
H = 16
DH = 28
DP = 32
HP = H * DP
NB = 2
NH = NB * H
NG = NH // 4
TQ = 512
NQ = S // TQ
GR = 16
CK = 256
D3 = 3 * D

_QSCALE = (DH ** -0.5) * math.log2(math.e)


def _kernel(xt_ref, wa_ref, wb_ref, woa_ref, wob_ref, gw_ref, o_ref,
            wt_scr, wop_scr, wot_scr, raw_scr, k_scr, qt_scr, vt_scr, g_scr, s_scr, ot_scr):
    f32 = jnp.float32
    bf16 = jnp.bfloat16
    w_refs = (wa_ref, wb_ref)
    wo_refs = (woa_ref, wob_ref)

    r32 = jax.lax.broadcasted_iota(jnp.int32, (DP, D), 0)
    for br in range(NB):
        wt_scr[br, 0:D3, :] = w_refs[br][...].T
        wt_scr[br, D3:D3 + GR, :] = jnp.broadcast_to(gw_ref[...], (GR, D))
        wop_scr[0:D, :] = wo_refs[br][...].astype(f32)
        wop_scr[D:D + 8, :] = jnp.zeros((8, D), f32)
        blks = []
        for h in range(H):
            blks.append(jnp.where(r32 < DH, wop_scr[h * DH:h * DH + DP, :], 0.0))
        wot_scr[:, br * HP:(br + 1) * HP] = jnp.concatenate(blks, axis=0).T.astype(bf16)

    rq = jax.lax.broadcasted_iota(jnp.int32, (DP, TQ), 0)
    for qb in range(NQ):
        cols = slice(qb * TQ, (qb + 1) * TQ)
        xt = xt_ref[:, cols]
        for br in range(NB):
            nrows = D3 + GR if br == 0 else D3
            raw = jnp.dot(wt_scr[br, 0:nrows, :], xt, preferred_element_type=f32)
            raw_scr[br, 0:nrows, :] = raw
            if br == 1:
                raw_scr[br, D3:D3 + 8, :] = jnp.zeros((8, TQ), f32)
            for gg in range(4):
                kb = []
                for j in range(4):
                    h = gg * 4 + j
                    q = raw_scr[br, h * DH:h * DH + DP, :]
                    qt_scr[br * 4 + gg, qb, j * DP:(j + 1) * DP, :] = (
                        jnp.where(rq < DH, q * _QSCALE, 0.0).astype(bf16))
                    k = raw_scr[br, D + h * DH:D + h * DH + DP, :]
                    kb.append(jnp.where(rq < DH, k, 0.0))
                    v = raw_scr[br, 2 * D + h * DH:2 * D + h * DH + DP, :]
                    v = jnp.where(rq < DH, v, jnp.where(rq == DH, 1.0, 0.0))
                    vt_scr[br * H + h, :, cols] = v.astype(bf16)
                k_scr[br * 4 + gg, cols, :] = jnp.concatenate(kb, axis=0).T.astype(bf16)
        gate = jax.nn.sigmoid(raw_scr[0, D3:D3 + 8, :])
        g_scr[0, qb] = gate
        g_scr[1, qb] = 1.0 - gate

    qrow = jax.lax.broadcasted_iota(jnp.int32, (128, TQ), 0) // DP

    def qm_of(hh, qb):
        qt = qt_scr[hh // 4, qb]
        return jnp.where(qrow == hh % 4, qt, jnp.zeros_like(qt))

    def head_step(hh, ms, do_qk):
        hn = hh + 1
        g = hn // 4
        r0 = pl.multiple_of(hh * DP, DP)
        out_ms = []
        for qb in range(NQ):
            if do_qk:
                qm = qm_of(hn, qb)
            m_c = ms[qb]
            m8 = None
            acc = None
            for c in range(S // CK):
                rows = slice(c * CK, (c + 1) * CK)
                if do_qk:
                    s = jnp.dot(k_scr[g, rows, :], qm, preferred_element_type=f32)
                p = jnp.exp2(s_scr[qb, rows, :] - m_c).astype(bf16)
                if do_qk:
                    s_scr[qb, rows, :] = s
                    mc = jnp.max(s.reshape(CK // 8, 8, TQ), axis=0)
                    m8 = mc if m8 is None else jnp.maximum(m8, mc)
                o = jnp.dot(vt_scr[hh, :, rows], p, preferred_element_type=f32)
                acc = o if acc is None else acc + o
            l = acc[DH:DH + 1, :]
            gf = g_scr[hh // H, qb][0:1, :]
            ot_scr[qb, pl.ds(r0, DP), :] = (acc * (gf / l)).astype(bf16)
            if do_qk:
                out_ms.append(jnp.max(m8, axis=0, keepdims=True))
        return tuple(out_ms)

    ms0 = []
    for qb in range(NQ):
        s = jnp.dot(k_scr[0], qm_of(0, qb), preferred_element_type=f32)
        s_scr[qb] = s
        ms0.append(jnp.max(s, axis=0, keepdims=True))
    ms = jax.lax.fori_loop(0, NH - 1, lambda hh, ms: head_step(hh, ms, True), tuple(ms0))
    head_step(NH - 1, ms, False)

    for qb in range(NQ):
        ot = jnp.dot(wot_scr[...], ot_scr[qb], preferred_element_type=f32)
        o_ref[:, qb * TQ:(qb + 1) * TQ] = ot.astype(o_ref.dtype)


@jax.jit
def pallas_gated_mix__mha_block__mha_block__prompt_kernel(
    A_x: jax.Array,
    A_wqkv: jax.Array,
    A_wo: jax.Array,
    B_x: jax.Array,
    B_wqkv: jax.Array,
    B_wo: jax.Array,
    gate_w: jax.Array,
):
    xt = A_x.reshape(S, D).T
    out_t = pl.pallas_call(
        _kernel,
        out_shape=jax.ShapeDtypeStruct((D, S), jnp.bfloat16),
        scratch_shapes=[
            pltpu.VMEM((NB, D3 + GR, D), jnp.bfloat16),
            pltpu.VMEM((D + 8, D), jnp.float32),
            pltpu.VMEM((D, NB * HP), jnp.bfloat16),
            pltpu.VMEM((NB, D3 + GR, TQ), jnp.float32),
            pltpu.VMEM((NG, S, 128), jnp.bfloat16),
            pltpu.VMEM((NG, NQ, 128, TQ), jnp.bfloat16),
            pltpu.VMEM((NH, DP, S), jnp.bfloat16),
            pltpu.VMEM((NB, NQ, 8, TQ), jnp.float32),
            pltpu.VMEM((NQ, S, TQ), jnp.float32),
            pltpu.VMEM((NQ, NH * DP, TQ), jnp.bfloat16),
        ],
        compiler_params=pltpu.CompilerParams(vmem_limit_bytes=100 * 1024 * 1024),
    )(xt, A_wqkv, B_wqkv, A_wo, B_wo, gate_w.reshape(1, D))
    return out_t.T.reshape(1, S, D)
```

```python
import math

import jax
import jax.numpy as jnp
import jax.experimental.pallas as pl
import jax.experimental.pallas.tpu as pltpu

S = 2048
D = 448
H = 16
DH = 28
DP = 32
HP = H * DP
NB = 2
NH = NB * H
NG = NH // 4
TQ = 512
NQ = S // TQ
GR = 16
CK = 256
D3 = 3 * D

_QSCALE = (DH ** -0.5) * math.log2(math.e)


def _kernel(xt_hbm, wa_hbm, wb_hbm, woa_hbm, wob_hbm, gw_ref, o_hbm,
            xt_ref, w_ref, wo_ref, o_ref, in_sems, out_sems,
            wt_scr, wop_scr, wot_scr, raw_scr, k_scr, qt_scr, vt_scr, g_scr, s_scr, ot_scr):
    f32 = jnp.float32
    bf16 = jnp.bfloat16

    w_cp = [pltpu.make_async_copy(src, w_ref.at[br], in_sems.at[br])
            for br, src in enumerate((wa_hbm, wb_hbm))]
    x_cp = [pltpu.make_async_copy(xt_hbm.at[:, qb * TQ:(qb + 1) * TQ],
                                  xt_ref.at[:, qb * TQ:(qb + 1) * TQ], in_sems.at[2 + qb])
            for qb in range(NQ)]
    wo_cp = [pltpu.make_async_copy(src, wo_ref.at[br], in_sems.at[2 + NQ + br])
             for br, src in enumerate((woa_hbm, wob_hbm))]
    w_cp[0].start()
    x_cp[0].start()
    w_cp[1].start()
    for qb in range(1, NQ):
        x_cp[qb].start()
    for br in range(NB):
        wo_cp[br].start()

    rq = jax.lax.broadcasted_iota(jnp.int32, (DP, TQ), 0)
    for qb in range(NQ):
        cols = slice(qb * TQ, (qb + 1) * TQ)
        for br in range(NB):
            if qb == 0:
                w_cp[br].wait()
                wt_scr[br, 0:D3, :] = w_ref[br].T
                wt_scr[br, D3:D3 + GR, :] = jnp.broadcast_to(gw_ref[...], (GR, D))
            if br == 0:
                x_cp[qb].wait()
            xt = xt_ref[:, cols]
            nrows = D3 + GR if br == 0 else D3
            raw = jnp.dot(wt_scr[br, 0:nrows, :], xt, preferred_element_type=f32)
            raw_scr[br, 0:nrows, :] = raw
            if br == 1:
                raw_scr[br, D3:D3 + 8, :] = jnp.zeros((8, TQ), f32)
            for gg in range(4):
                kb = []
                for j in range(4):
                    h = gg * 4 + j
                    q = raw_scr[br, h * DH:h * DH + DP, :]
                    qt_scr[br * 4 + gg, qb, j * DP:(j + 1) * DP, :] = (
                        jnp.where(rq < DH, q * _QSCALE, 0.0).astype(bf16))
                    k = raw_scr[br, D + h * DH:D + h * DH + DP, :]
                    kb.append(jnp.where(rq < DH, k, 0.0))
                    v = raw_scr[br, 2 * D + h * DH:2 * D + h * DH + DP, :]
                    v = jnp.where(rq < DH, v, jnp.where(rq == DH, 1.0, 0.0))
                    vt_scr[br * H + h, :, cols] = v.astype(bf16)
                k_scr[br * 4 + gg, cols, :] = jnp.concatenate(kb, axis=0).T.astype(bf16)
        gate = jax.nn.sigmoid(raw_scr[0, D3:D3 + 8, :])
        g_scr[0, qb] = gate
        g_scr[1, qb] = 1.0 - gate

    r32 = jax.lax.broadcasted_iota(jnp.int32, (DP, D), 0)
    for br in range(NB):
        wo_cp[br].wait()
        wop_scr[0:D, :] = wo_ref[br].astype(f32)
        wop_scr[D:D + 8, :] = jnp.zeros((8, D), f32)
        blks = []
        for h in range(H):
            blks.append(jnp.where(r32 < DH, wop_scr[h * DH:h * DH + DP, :], 0.0))
        wot_scr[:, br * HP:(br + 1) * HP] = jnp.concatenate(blks, axis=0).T.astype(bf16)

    qrow = jax.lax.broadcasted_iota(jnp.int32, (128, TQ), 0) // DP

    def qm_of(hh, qb):
        qt = qt_scr[hh // 4, qb]
        return jnp.where(qrow == hh % 4, qt, jnp.zeros_like(qt))

    def head_step(hh, ms, do_qk):
        hn = hh + 1
        g = hn // 4
        r0 = pl.multiple_of(hh * DP, DP)
        out_ms = []
        for qb in range(NQ):
            if do_qk:
                qm = qm_of(hn, qb)
            m_c = ms[qb]
            m8 = None
            acc = None
            for c in range(S // CK):
                rows = slice(c * CK, (c + 1) * CK)
                if do_qk:
                    s = jnp.dot(k_scr[g, rows, :], qm, preferred_element_type=f32)
                p = jnp.exp2(s_scr[qb, rows, :] - m_c).astype(bf16)
                if do_qk:
                    s_scr[qb, rows, :] = s
                    mc = jnp.max(s.reshape(CK // 8, 8, TQ), axis=0)
                    m8 = mc if m8 is None else jnp.maximum(m8, mc)
                o = jnp.dot(vt_scr[hh, :, rows], p, preferred_element_type=f32)
                acc = o if acc is None else acc + o
            l = acc[DH:DH + 1, :]
            gf = g_scr[hh // H, qb][0:1, :]
            ot_scr[qb, pl.ds(r0, DP), :] = (acc * (gf / l)).astype(bf16)
            if do_qk:
                out_ms.append(jnp.max(m8, axis=0, keepdims=True))
        return tuple(out_ms)

    ms0 = []
    for qb in range(NQ):
        s = jnp.dot(k_scr[0], qm_of(0, qb), preferred_element_type=f32)
        s_scr[qb] = s
        ms0.append(jnp.max(s, axis=0, keepdims=True))
    ms = jax.lax.fori_loop(0, NH - 1, lambda hh, ms: head_step(hh, ms, True), tuple(ms0))
    head_step(NH - 1, ms, False)

    o_cp = []
    for qb in range(NQ):
        cols = slice(qb * TQ, (qb + 1) * TQ)
        ot = jnp.dot(wot_scr[...], ot_scr[qb], preferred_element_type=f32)
        o_ref[:, cols] = ot.astype(o_ref.dtype)
        cp = pltpu.make_async_copy(o_ref.at[:, cols], o_hbm.at[:, cols], out_sems.at[qb])
        cp.start()
        o_cp.append(cp)
    for cp in o_cp:
        cp.wait()


@jax.jit
def pallas_gated_mix__mha_block__mha_block__prompt_kernel(
    A_x: jax.Array,
    A_wqkv: jax.Array,
    A_wo: jax.Array,
    B_x: jax.Array,
    B_wqkv: jax.Array,
    B_wo: jax.Array,
    gate_w: jax.Array,
):
    xt = A_x.reshape(S, D).T
    out_t = pl.pallas_call(
        _kernel,
        out_shape=jax.ShapeDtypeStruct((D, S), jnp.bfloat16),
        in_specs=[pl.BlockSpec(memory_space=pl.ANY)] * 5 + [pl.BlockSpec(memory_space=pltpu.VMEM)],
        out_specs=pl.BlockSpec(memory_space=pl.ANY),
        scratch_shapes=[
            pltpu.VMEM((D, S), jnp.bfloat16),
            pltpu.VMEM((NB, D, D3), jnp.bfloat16),
            pltpu.VMEM((NB, D, D), jnp.bfloat16),
            pltpu.VMEM((D, S), jnp.bfloat16),
            pltpu.SemaphoreType.DMA((2 + NQ + 2,)),
            pltpu.SemaphoreType.DMA((NQ,)),
            pltpu.VMEM((NB, D3 + GR, D), jnp.bfloat16),
            pltpu.VMEM((D + 8, D), jnp.float32),
            pltpu.VMEM((D, NB * HP), jnp.bfloat16),
            pltpu.VMEM((NB, D3 + GR, TQ), jnp.float32),
            pltpu.VMEM((NG, S, 128), jnp.bfloat16),
            pltpu.VMEM((NG, NQ, 128, TQ), jnp.bfloat16),
            pltpu.VMEM((NH, DP, S), jnp.bfloat16),
            pltpu.VMEM((NB, NQ, 8, TQ), jnp.float32),
            pltpu.VMEM((NQ, S, TQ), jnp.float32),
            pltpu.VMEM((NQ, NH * DP, TQ), jnp.bfloat16),
        ],
        compiler_params=pltpu.CompilerParams(vmem_limit_bytes=100 * 1024 * 1024),
    )(xt, A_wqkv, B_wqkv, A_wo, B_wo, gate_w.reshape(1, D))
    return out_t.T.reshape(1, S, D)
```

```python
import math

import jax
import jax.numpy as jnp
import jax.experimental.pallas as pl
import jax.experimental.pallas.tpu as pltpu

S = 2048
D = 448
H = 16
DH = 28
DP = 32
HP = H * DP
NB = 2
NH = NB * H
NG = NH // 4
TQ = 512
NQ = S // TQ
GR = 16
CK = 128
D3 = 3 * D
LAG = 1

_QSCALE = (DH ** -0.5) * math.log2(math.e)


def _kernel(xt_hbm, wa_hbm, wb_hbm, woa_hbm, wob_hbm, gw_ref, o_hbm,
            xt_ref, w_ref, wo_ref, o_ref, in_sems, out_sems,
            wt_scr, wop_scr, wot_scr, raw_scr, k_scr, qt_scr, vt_scr, g_scr, s_scr, ot_scr, o3_scr):
    f32 = jnp.float32
    bf16 = jnp.bfloat16

    wparts = [(0, 512), (512, 1024), (1024, D3)]
    wa_cp = [pltpu.make_async_copy(wa_hbm.at[:, lo:hi], w_ref.at[0, :, lo:hi], in_sems.at[i])
             for i, (lo, hi) in enumerate(wparts)]
    wb_cp = pltpu.make_async_copy(wb_hbm, w_ref.at[1], in_sems.at[3])

    def x_cp(qb):
        c0 = pl.multiple_of(qb * TQ, TQ)
        return pltpu.make_async_copy(xt_hbm.at[:, pl.ds(c0, TQ)], xt_ref.at[qb],
                                     in_sems.at[4 + qb])

    wo_cp = [pltpu.make_async_copy(src, wo_ref.at[br], in_sems.at[4 + NQ + br])
             for br, src in enumerate((woa_hbm, wob_hbm))]
    wa_cp[0].start()
    x_cp(0).start()
    wa_cp[1].start()
    wa_cp[2].start()
    wb_cp.start()
    for qb in range(1, NQ):
        x_cp(qb).start()
    for br in range(NB):
        wo_cp[br].start()

    rq = jax.lax.broadcasted_iota(jnp.int32, (DP, TQ), 0)

    def relayout(qb, br):
        r0 = pl.multiple_of(qb * TQ, TQ)
        for gg in range(4):
            kb = []
            for j in range(4):
                h = gg * 4 + j
                q = raw_scr[h * DH:h * DH + DP, :]
                qt_scr[br * 4 + gg, qb, j * DP:(j + 1) * DP, :] = (
                    jnp.where(rq < DH, q * _QSCALE, 0.0).astype(bf16))
                k = raw_scr[D + h * DH:D + h * DH + DP, :]
                kb.append(jnp.where(rq < DH, k, 0.0))
                v = raw_scr[2 * D + h * DH:2 * D + h * DH + DP, :]
                v = jnp.where(rq < DH, v, jnp.where(rq == DH, 1.0, 0.0))
                vt_scr[br * H + h, qb] = v.astype(bf16)
            k_scr[br * 4 + gg, pl.ds(r0, TQ), :] = jnp.concatenate(kb, axis=0).T.astype(bf16)
        gate = jax.nn.sigmoid(raw_scr[D3:D3 + 8, :])
        g_scr[br, qb] = jnp.where(br == 0, gate, 1.0 - gate)

    gwb = jnp.broadcast_to(gw_ref[...], (GR, D))
    wt_scr[0, D3:D3 + GR, :] = gwb
    wt_scr[1, D3:D3 + GR, :] = gwb
    for i, (lo, hi) in enumerate(wparts):
        wa_cp[i].wait()
        if i == 0:
            x_cp(0).wait()
        if i == len(wparts) - 1:
            wb_cp.wait()
        wt_scr[0, lo:hi, :] = w_ref[0, :, lo:hi].T
        hi2 = hi + GR if i == len(wparts) - 1 else hi
        raw_scr[lo:hi2, :] = jnp.dot(wt_scr[0, lo:hi2, :], xt_ref[0], preferred_element_type=f32)
    wt_scr[1, 0:D3, :] = w_ref[1].T
    relayout(0, 0)

    def proj(it, carry):
        qb = it // NB
        br = it % NB

        @pl.when(br == 0)
        def _():
            x_cp(qb).wait()

        raw_scr[...] = jnp.dot(wt_scr[br], xt_ref[qb], preferred_element_type=f32)
        relayout(qb, br)
        return carry

    jax.lax.fori_loop(1, NQ * NB, proj, 0)

    r32 = jax.lax.broadcasted_iota(jnp.int32, (DP, D), 0)
    for br in range(NB):
        wo_cp[br].wait()
        wop_scr[0:D, :] = wo_ref[br].astype(f32)
        wop_scr[D:D + 8, :] = jnp.zeros((8, D), f32)
        blks = []
        for h in range(H):
            blks.append(jnp.where(r32 < DH, wop_scr[h * DH:h * DH + DP, :], 0.0))
        wot_scr[:, br * HP:(br + 1) * HP] = jnp.concatenate(blks, axis=0).T.astype(bf16)

    qrow = jax.lax.broadcasted_iota(jnp.int32, (128, TQ), 0) // DP

    def qm_of(hh, qb):
        qt = qt_scr[hh // 4, qb]
        return jnp.where(qrow == hh % 4, qt, jnp.zeros_like(qt))

    def head_step(hh, ms, do_qk):
        hn = hh + 1
        g = hn // 4
        r0 = pl.multiple_of(hh * DP, DP)
        nc = S // CK
        cpq = TQ // CK
        steps = [(qb, c) for qb in range(NQ) for c in range(nc)]
        st = dict(qm=None, m8=None, acc=None)
        out_ms = []

        def do_pv(qb, c):
            rows = slice(c * CK, (c + 1) * CK)
            p = jnp.exp2(s_scr[qb, rows, :] - ms[qb]).astype(bf16)
            vt = vt_scr[hh, c // cpq, :, (c % cpq) * CK:(c % cpq + 1) * CK]
            o = jnp.dot(vt, p, preferred_element_type=f32)
            st['acc'] = o if c == 0 else st['acc'] + o
            if c == nc - 1:
                acc = st['acc']
                l = acc[DH:DH + 1, :]
                gf = g_scr[hh // H, qb][0:1, :]
                ot_scr[qb, pl.ds(r0, DP), :] = (acc * (gf / l)).astype(bf16)

        def do_qk_chunk(qb, c):
            rows = slice(c * CK, (c + 1) * CK)
            if c == 0:
                st['qm'] = qm_of(hn, qb)
            s = jnp.dot(k_scr[g, rows, :], st['qm'], preferred_element_type=f32)
            s_scr[qb, rows, :] = s
            mc = jnp.max(s.reshape(CK // 8, 8, TQ), axis=0)
            st['m8'] = mc if c == 0 else jnp.maximum(st['m8'], mc)
            if c == nc - 1:
                out_ms.append(jnp.max(st['m8'], axis=0, keepdims=True))

        for t in range(-LAG, len(steps)):
            if t + LAG < len(steps):
                do_pv(*steps[t + LAG])
            if do_qk and t >= 0:
                do_qk_chunk(*steps[t])
        return tuple(out_ms)

    ms0 = []
    for qb in range(NQ):
        s = jnp.dot(k_scr[0], qm_of(0, qb), preferred_element_type=f32)
        s_scr[qb] = s
        ms0.append(jnp.max(s, axis=0, keepdims=True))
    ms = jax.lax.fori_loop(0, NH - 1, lambda hh, ms: head_step(hh, ms, True), tuple(ms0))

    hl = NH - 1
    k7 = (NH - 4) * DP
    npc = 7
    rp = D // npc
    nc = S // CK
    cpq = TQ // CK
    o_cp = []

    def finish(qb):
        cols = slice(qb * TQ, (qb + 1) * TQ)
        ot = o3_scr[qb % 2] + jnp.dot(wot_scr[:, k7:], ot_scr[qb, k7:, :],
                                      preferred_element_type=f32)
        o_ref[:, cols] = ot.astype(o_ref.dtype)
        cp = pltpu.make_async_copy(o_ref.at[:, cols], o_hbm.at[:, cols], out_sems.at[qb])
        cp.start()
        o_cp.append(cp)

    for qb in range(NQ):
        acc = None
        for i in range(npc):
            o3_scr[qb % 2, i * rp:(i + 1) * rp, :] = jnp.dot(
                wot_scr[i * rp:(i + 1) * rp, 0:k7], ot_scr[qb, 0:k7, :],
                preferred_element_type=f32)
            if i == 0 and qb > 0:
                finish(qb - 1)
            for c in range(i * nc // npc, (i + 1) * nc // npc):
                rows = slice(c * CK, (c + 1) * CK)
                p = jnp.exp2(s_scr[qb, rows, :] - ms[qb]).astype(bf16)
                vt = vt_scr[hl, c // cpq, :, (c % cpq) * CK:(c % cpq + 1) * CK]
                o = jnp.dot(vt, p, preferred_element_type=f32)
                acc = o if acc is None else acc + o
        l = acc[DH:DH + 1, :]
        gf = g_scr[1, qb][0:1, :]
        ot_scr[qb, hl * DP:(hl + 1) * DP, :] = (acc * (gf / l)).astype(bf16)
    finish(NQ - 1)
    for cp in o_cp:
        cp.wait()


@jax.jit
def pallas_gated_mix__mha_block__mha_block__prompt_kernel(
    A_x: jax.Array,
    A_wqkv: jax.Array,
    A_wo: jax.Array,
    B_x: jax.Array,
    B_wqkv: jax.Array,
    B_wo: jax.Array,
    gate_w: jax.Array,
):
    xt = A_x.reshape(S, D).T
    out_t = pl.pallas_call(
        _kernel,
        out_shape=jax.ShapeDtypeStruct((D, S), jnp.bfloat16),
        in_specs=[pl.BlockSpec(memory_space=pl.ANY)] * 5 + [pl.BlockSpec(memory_space=pltpu.VMEM)],
        out_specs=pl.BlockSpec(memory_space=pl.ANY),
        scratch_shapes=[
            pltpu.VMEM((NQ, D, TQ), jnp.bfloat16),
            pltpu.VMEM((NB, D, D3), jnp.bfloat16),
            pltpu.VMEM((NB, D, D), jnp.bfloat16),
            pltpu.VMEM((D, S), jnp.bfloat16),
            pltpu.SemaphoreType.DMA((4 + NQ + 2,)),
            pltpu.SemaphoreType.DMA((NQ,)),
            pltpu.VMEM((NB, D3 + GR, D), jnp.bfloat16),
            pltpu.VMEM((D + 8, D), jnp.float32),
            pltpu.VMEM((D, NB * HP), jnp.bfloat16),
            pltpu.VMEM((D3 + GR, TQ), jnp.float32),
            pltpu.VMEM((NG, S, 128), jnp.bfloat16),
            pltpu.VMEM((NG, NQ, 128, TQ), jnp.bfloat16),
            pltpu.VMEM((NH, NQ, DP, TQ), jnp.bfloat16),
            pltpu.VMEM((NB, NQ, 8, TQ), jnp.float32),
            pltpu.VMEM((NQ, S, TQ), jnp.float32),
            pltpu.VMEM((NQ, NH * DP, TQ), jnp.bfloat16),
            pltpu.VMEM((2, D, TQ), jnp.float32),
        ],
        compiler_params=pltpu.CompilerParams(vmem_limit_bytes=100 * 1024 * 1024),
    )(xt, A_wqkv, B_wqkv, A_wo, B_wo, gate_w.reshape(1, D))
    return out_t.T.reshape(1, S, D)
```

```python
import math

import jax
import jax.numpy as jnp
import jax.experimental.pallas as pl
import jax.experimental.pallas.tpu as pltpu

S = 2048
D = 448
H = 16
DH = 28
DP = 32
HP = H * DP
NB = 2
NH = NB * H
NG = NH // 4
TQ = 512
NQ = S // TQ
GR = 16
CK = 128
D3 = 3 * D
LAG = 1
HPI = 2

_QSCALE = (DH ** -0.5) * math.log2(math.e)


def _kernel(xt_hbm, wa_hbm, wb_hbm, woa_hbm, wob_hbm, gw_ref, o_hbm,
            xt_ref, w_ref, wo_ref, o_ref, in_sems, out_sems,
            wt_scr, wop_scr, wot_scr, raw_scr, k_scr, qt_scr, vt_scr, g_scr, s_scr, ot_scr, o3_scr):
    f32 = jnp.float32
    bf16 = jnp.bfloat16

    wparts = [(0, 512), (512, 1024), (1024, D3)]
    wa_cp = [pltpu.make_async_copy(wa_hbm.at[:, lo:hi], w_ref.at[0, :, lo:hi], in_sems.at[i])
             for i, (lo, hi) in enumerate(wparts)]
    wb_cp = pltpu.make_async_copy(wb_hbm, w_ref.at[1], in_sems.at[3])

    def x_cp(qb):
        c0 = pl.multiple_of(qb * TQ, TQ)
        return pltpu.make_async_copy(xt_hbm.at[:, pl.ds(c0, TQ)], xt_ref.at[qb],
                                     in_sems.at[4 + qb])

    wo_cp = [pltpu.make_async_copy(src, wo_ref.at[br], in_sems.at[4 + NQ + br])
             for br, src in enumerate((woa_hbm, wob_hbm))]
    wa_cp[0].start()
    x_cp(0).start()
    wa_cp[1].start()
    wa_cp[2].start()
    wb_cp.start()
    for qb in range(1, NQ):
        x_cp(qb).start()
    for br in range(NB):
        wo_cp[br].start()

    rq = jax.lax.broadcasted_iota(jnp.int32, (DP, TQ), 0)

    def relayout(qb, br):
        r0 = pl.multiple_of(qb * TQ, TQ)
        for gg in range(4):
            kb = []
            for j in range(4):
                h = gg * 4 + j
                q = raw_scr[h * DH:h * DH + DP, :]
                qt_scr[br * 4 + gg, qb, j * DP:(j + 1) * DP, :] = (
                    jnp.where(rq < DH, q * _QSCALE, 0.0).astype(bf16))
                k = raw_scr[D + h * DH:D + h * DH + DP, :]
                kb.append(jnp.where(rq < DH, k, 0.0))
                v = raw_scr[2 * D + h * DH:2 * D + h * DH + DP, :]
                v = jnp.where(rq < DH, v, jnp.where(rq == DH, 1.0, 0.0))
                vt_scr[br * H + h, qb] = v.astype(bf16)
            k_scr[br * 4 + gg, pl.ds(r0, TQ), :] = jnp.concatenate(kb, axis=0).T.astype(bf16)
        gate = jax.nn.sigmoid(raw_scr[D3:D3 + 8, :])
        g_scr[br, qb] = jnp.where(br == 0, gate, 1.0 - gate)

    gwb = jnp.broadcast_to(gw_ref[...].reshape(1, D), (GR, D))
    wt_scr[0, D3:D3 + GR, :] = gwb
    wt_scr[1, D3:D3 + GR, :] = gwb
    for i, (lo, hi) in enumerate(wparts):
        wa_cp[i].wait()
        if i == 0:
            x_cp(0).wait()
        if i == len(wparts) - 1:
            wb_cp.wait()
        wt_scr[0, lo:hi, :] = w_ref[0, :, lo:hi].T
        hi2 = hi + GR if i == len(wparts) - 1 else hi
        raw_scr[lo:hi2, :] = jnp.dot(wt_scr[0, lo:hi2, :], xt_ref[0], preferred_element_type=f32)
    wt_scr[1, 0:D3, :] = w_ref[1].T
    relayout(0, 0)

    def proj(it, carry):
        qb = it // NB
        br = it % NB

        @pl.when(br == 0)
        def _():
            x_cp(qb).wait()

        raw_scr[...] = jnp.dot(wt_scr[br], xt_ref[qb], preferred_element_type=f32)
        relayout(qb, br)
        return carry

    jax.lax.fori_loop(1, NQ * NB, proj, 0)

    r32 = jax.lax.broadcasted_iota(jnp.int32, (DP, D), 0)
    for br in range(NB):
        wo_cp[br].wait()
        wop_scr[0:D, :] = wo_ref[br].astype(f32)
        wop_scr[D:D + 8, :] = jnp.zeros((8, D), f32)
        blks = []
        for h in range(H):
            blks.append(jnp.where(r32 < DH, wop_scr[h * DH:h * DH + DP, :], 0.0))
        wot_scr[:, br * HP:(br + 1) * HP] = jnp.concatenate(blks, axis=0).T.astype(bf16)

    qrow = jax.lax.broadcasted_iota(jnp.int32, (128, TQ), 0) // DP

    def qm_of(hh, qb):
        qt = qt_scr[hh // 4, qb]
        return jnp.where(qrow == hh % 4, qt, jnp.zeros_like(qt))

    nc = S // CK
    cpq = TQ // CK

    def pv_chunk(hh, buf, m, c, acc):
        rows = slice(c * CK, (c + 1) * CK)
        p = jnp.exp2(s_scr[buf, rows, :] - m).astype(bf16)
        vt = vt_scr[hh, c // cpq, :, (c % cpq) * CK:(c % cpq + 1) * CK]
        o = jnp.dot(vt, p, preferred_element_type=f32)
        return o if acc is None else acc + o

    def pv_finish(hh, qb, acc):
        r0 = hh * DP if isinstance(hh, int) else pl.multiple_of(hh * DP, DP)
        l = acc[DH:DH + 1, :]
        gf = g_scr[hh // H, qb][0:1, :]
        ot_scr[qb, pl.ds(r0, DP), :] = (acc * (gf / l)).astype(bf16)

    def body(i, ms):
        steps = [(u, qb, c) for u in range(HPI) for qb in range(NQ) for c in range(nc)]
        st = dict(qm=None, m8=None, acc=None)
        out_ms = []

        def do_pv(u, qb, c):
            hh = i * HPI + u
            buf = u * NQ + qb
            st['acc'] = pv_chunk(hh, buf, ms[buf], c, None if c == 0 else st['acc'])
            if c == nc - 1:
                pv_finish(hh, qb, st['acc'])

        def do_qk(u, qb, c):
            hn = (i + 1) * HPI + u
            buf = u * NQ + qb
            rows = slice(c * CK, (c + 1) * CK)
            if c == 0:
                st['qm'] = qm_of(hn, qb)
            s = jnp.dot(k_scr[hn // 4, rows, :], st['qm'], preferred_element_type=f32)
            s_scr[buf, rows, :] = s
            mc = jnp.max(s.reshape(CK // 8, 8, TQ), axis=0)
            st['m8'] = mc if c == 0 else jnp.maximum(st['m8'], mc)
            if c == nc - 1:
                out_ms.append(jnp.max(st['m8'], axis=0, keepdims=True))

        for t in range(-LAG, len(steps)):
            if t + LAG < len(steps):
                do_pv(*steps[t + LAG])
            if t >= 0:
                do_qk(*steps[t])
        return tuple(out_ms)

    ms0 = []
    for u in range(HPI):
        for qb in range(NQ):
            s = jnp.dot(k_scr[0], qm_of(u, qb), preferred_element_type=f32)
            s_scr[u * NQ + qb] = s
            ms0.append(jnp.max(s, axis=0, keepdims=True))
    ms = jax.lax.fori_loop(0, NH // HPI - 1, body, tuple(ms0))

    k7 = (NH - 4) * DP
    npc = 7
    rp = D // npc
    o_cp = []

    def finish(qb):
        cols = slice(qb * TQ, (qb + 1) * TQ)
        ot = o3_scr[qb % 2] + jnp.dot(wot_scr[:, k7:], ot_scr[qb, k7:, :],
                                      preferred_element_type=f32)
        o_ref[:, cols] = ot.astype(o_ref.dtype)
        cp = pltpu.make_async_copy(o_ref.at[:, cols], o_hbm.at[:, cols], out_sems.at[qb])
        cp.start()
        o_cp.append(cp)

    mq = D // 4
    pieces = [(mi, kt) for mi in range(4) for kt in range(k7 // 128)]
    for qb in range(NQ):
        work = [(u, c) for u in range(HPI) for c in range(nc)]
        acc = None
        for i, (mi, kt) in enumerate(pieces):
            rs = slice(mi * mq, (mi + 1) * mq)
            ks = slice(kt * 128, (kt + 1) * 128)
            part = jnp.dot(wot_scr[rs, ks], ot_scr[qb, ks, :], preferred_element_type=f32)
            if kt == 0:
                o3_scr[qb % 2, rs, :] = part
            else:
                o3_scr[qb % 2, rs, :] = o3_scr[qb % 2, rs, :] + part
            if i == 2 and qb > 0:
                finish(qb - 1)
            lo, hi = i * len(work) // len(pieces), (i + 1) * len(work) // len(pieces)
            for (u, c) in work[lo:hi]:
                hh = NH - HPI + u
                buf = u * NQ + qb
                acc = pv_chunk(hh, buf, ms[buf], c, None if c == 0 else acc)
                if c == nc - 1:
                    pv_finish(hh, qb, acc)
    finish(NQ - 1)
    for cp in o_cp:
        cp.wait()


@jax.jit
def pallas_gated_mix__mha_block__mha_block__prompt_kernel(
    A_x: jax.Array,
    A_wqkv: jax.Array,
    A_wo: jax.Array,
    B_x: jax.Array,
    B_wqkv: jax.Array,
    B_wo: jax.Array,
    gate_w: jax.Array,
):
    xt = A_x.reshape(S, D).T
    out_t = pl.pallas_call(
        _kernel,
        out_shape=jax.ShapeDtypeStruct((D, S), jnp.bfloat16),
        in_specs=[pl.BlockSpec(memory_space=pl.ANY)] * 5 + [pl.BlockSpec(memory_space=pltpu.VMEM)],
        out_specs=pl.BlockSpec(memory_space=pl.ANY),
        scratch_shapes=[
            pltpu.VMEM((NQ, D, TQ), jnp.bfloat16),
            pltpu.VMEM((NB, D, D3), jnp.bfloat16),
            pltpu.VMEM((NB, D, D), jnp.bfloat16),
            pltpu.VMEM((D, S), jnp.bfloat16),
            pltpu.SemaphoreType.DMA((4 + NQ + 2,)),
            pltpu.SemaphoreType.DMA((NQ,)),
            pltpu.VMEM((NB, D3 + GR, D), jnp.bfloat16),
            pltpu.VMEM((D + 8, D), jnp.float32),
            pltpu.VMEM((D, NB * HP), jnp.bfloat16),
            pltpu.VMEM((D3 + GR, TQ), jnp.float32),
            pltpu.VMEM((NG, S, 128), jnp.bfloat16),
            pltpu.VMEM((NG, NQ, 128, TQ), jnp.bfloat16),
            pltpu.VMEM((NH, NQ, DP, TQ), jnp.bfloat16),
            pltpu.VMEM((NB, NQ, 8, TQ), jnp.float32),
            pltpu.VMEM((HPI * NQ, S, TQ), jnp.float32),
            pltpu.VMEM((NQ, NH * DP, TQ), jnp.bfloat16),
            pltpu.VMEM((2, D, TQ), jnp.float32),
        ],
        compiler_params=pltpu.CompilerParams(vmem_limit_bytes=100 * 1024 * 1024),
    )(xt, A_wqkv, B_wqkv, A_wo, B_wo, gate_w)
    return out_t.T.reshape(1, S, D)
```

```python
import math

import jax
import jax.numpy as jnp
import jax.experimental.pallas as pl
import jax.experimental.pallas.tpu as pltpu

S = 2048
D = 448
H = 16
DH = 28
DP = 32
NB = 2
NH = NB * H
NG = NH // 4
TQ = 512
NQ = S // TQ
GR = 16
CK = 128
D3 = 3 * D
LAG = 1
HPI = 2

_QSCALE = (DH ** -0.5) * math.log2(math.e)


def _kernel(xt_hbm, wa_hbm, wb_hbm, woa_hbm, wob_hbm, gw_ref, o_hbm,
            xt_ref, w_ref, wo_ref, o_ref, in_sems, out_sems,
            wt_scr, wot_scr, raw_scr, k_scr, qt_scr, vt_scr, g_scr, s_scr, ot_scr, o3_scr, otb_scr):
    f32 = jnp.float32
    bf16 = jnp.bfloat16

    wparts = [(0, 512), (512, 1024), (1024, D3)]
    wa_cp = [pltpu.make_async_copy(wa_hbm.at[:, lo:hi], w_ref.at[0, :, lo:hi], in_sems.at[i])
             for i, (lo, hi) in enumerate(wparts)]
    wb_cp = pltpu.make_async_copy(wb_hbm, w_ref.at[1], in_sems.at[3])

    def x_cp(qb):
        c0 = pl.multiple_of(qb * TQ, TQ)
        return pltpu.make_async_copy(xt_hbm.at[:, pl.ds(c0, TQ)], xt_ref.at[qb],
                                     in_sems.at[4 + qb])

    wo_cp = [pltpu.make_async_copy(src, wo_ref.at[br], in_sems.at[4 + NQ + br])
             for br, src in enumerate((woa_hbm, wob_hbm))]
    wa_cp[0].start()
    x_cp(0).start()
    wa_cp[1].start()
    wa_cp[2].start()
    wb_cp.start()
    for qb in range(1, NQ):
        x_cp(qb).start()
    for br in range(NB):
        wo_cp[br].start()

    rq = jax.lax.broadcasted_iota(jnp.int32, (DP, TQ), 0)

    def relayout(qb, br):
        r0 = pl.multiple_of(qb * TQ, TQ)
        for gg in range(4):
            kb = []
            for j in range(4):
                h = gg * 4 + j
                q = raw_scr[h * DH:h * DH + DP, :]
                qt_scr[br * 4 + gg, qb, j * DP:(j + 1) * DP, :] = (
                    jnp.where(rq < DH, q * _QSCALE, 0.0).astype(bf16))
                k = raw_scr[D + h * DH:D + h * DH + DP, :]
                kb.append(jnp.where(rq < DH, k, 0.0))
                v = raw_scr[2 * D + h * DH:2 * D + h * DH + DP, :]
                v = jnp.where(rq < DH, v, jnp.where(rq == DH, 1.0, 0.0))
                vt_scr[br * H + h, qb] = v.astype(bf16)
            k_scr[br * 4 + gg, pl.ds(r0, TQ), :] = jnp.concatenate(kb, axis=0).T.astype(bf16)
        gate = jax.nn.sigmoid(raw_scr[D3:D3 + 8, :])
        g_scr[br, qb] = jnp.where(br == 0, gate, 1.0 - gate)

    gwb = jnp.broadcast_to(gw_ref[...].reshape(1, D), (GR, D))
    wt_scr[0, D3:D3 + GR, :] = gwb
    wt_scr[1, D3:D3 + GR, :] = gwb
    for i, (lo, hi) in enumerate(wparts):
        wa_cp[i].wait()
        if i == 0:
            x_cp(0).wait()
        if i == len(wparts) - 1:
            wb_cp.wait()
        wt_scr[0, lo:hi, :] = w_ref[0, :, lo:hi].T
        hi2 = hi + GR if i == len(wparts) - 1 else hi
        raw_scr[lo:hi2, :] = jnp.dot(wt_scr[0, lo:hi2, :], xt_ref[0], preferred_element_type=f32)
    wt_scr[1, 0:D3, :] = w_ref[1].T
    relayout(0, 0)

    def proj(it, carry):
        qb = it // NB
        br = it % NB

        @pl.when(br == 0)
        def _():
            x_cp(qb).wait()

        raw_scr[...] = jnp.dot(wt_scr[br], xt_ref[qb], preferred_element_type=f32)
        relayout(qb, br)
        return carry

    jax.lax.fori_loop(1, NQ * NB, proj, 0)

    for br in range(NB):
        wo_cp[br].wait()
        wot_scr[:, br * D:(br + 1) * D] = wo_ref[br].T

    qrow = jax.lax.broadcasted_iota(jnp.int32, (128, TQ), 0) // DP

    def qm_of(hh, qb):
        qt = qt_scr[hh // 4, qb]
        return jnp.where(qrow == hh % 4, qt, jnp.zeros_like(qt))

    nc = S // CK
    cpq = TQ // CK

    def pv_chunk(hh, buf, m, c, acc):
        rows = slice(c * CK, (c + 1) * CK)
        p = jnp.exp2(s_scr[buf, rows, :] - m).astype(bf16)
        vt = vt_scr[hh, c // cpq, :, (c % cpq) * CK:(c % cpq + 1) * CK]
        o = jnp.dot(vt, p, preferred_element_type=f32)
        return o if acc is None else acc + o

    def pv_norm(hh, qb, acc):
        l = acc[DH:DH + 1, :]
        gf = g_scr[hh // H, qb][0:1, :]
        return acc[0:DH, :] * (gf / l)

    def pv_store(i, qb, outs):
        r0 = i * HPI * DH if isinstance(i, int) else pl.multiple_of(i * (HPI * DH), 8)
        ot_scr[qb, pl.ds(r0, HPI * DH), :] = jnp.concatenate(outs, axis=0)

    def body(i, ms):
        steps = [(u, qb, c) for qb in range(NQ) for u in range(HPI) for c in range(nc)]
        st = dict(qm=None, m8=None, acc=None, outs=[])
        out_ms = {}

        def do_pv(u, qb, c):
            hh = i * HPI + u
            buf = u * NQ + qb
            st['acc'] = pv_chunk(hh, buf, ms[buf], c, None if c == 0 else st['acc'])
            if c == nc - 1:
                st['outs'].append(pv_norm(hh, qb, st['acc']))
                if u == HPI - 1:
                    pv_store(i, qb, st['outs'])
                    st['outs'] = []

        def do_qk(u, qb, c):
            hn = (i + 1) * HPI + u
            buf = u * NQ + qb
            rows = slice(c * CK, (c + 1) * CK)
            if c == 0:
                st['qm'] = qm_of(hn, qb)
            s = jnp.dot(k_scr[hn // 4, rows, :], st['qm'], preferred_element_type=f32)
            s_scr[buf, rows, :] = s
            mc = jnp.max(s.reshape(CK // 8, 8, TQ), axis=0)
            st['m8'] = mc if c == 0 else jnp.maximum(st['m8'], mc)
            if c == nc - 1:
                out_ms[buf] = jnp.max(st['m8'], axis=0, keepdims=True)

        for t in range(-LAG, len(steps)):
            if t + LAG < len(steps):
                do_pv(*steps[t + LAG])
            if t >= 0:
                do_qk(*steps[t])
        return tuple(out_ms[b] for b in range(HPI * NQ))

    ms0 = []
    for u in range(HPI):
        for qb in range(NQ):
            s = jnp.dot(k_scr[0], qm_of(u, qb), preferred_element_type=f32)
            s_scr[u * NQ + qb] = s
            ms0.append(jnp.max(s, axis=0, keepdims=True))
    ms = jax.lax.fori_loop(0, NH // HPI - 1, body, tuple(ms0))

    k7 = 6 * 128
    o_cp = []

    def finish(qb):
        cols = slice(qb * TQ, (qb + 1) * TQ)
        ot = o3_scr[qb % 2] + jnp.dot(wot_scr[:, k7:], ot_scr[qb, k7:, :].astype(bf16),
                                      preferred_element_type=f32)
        o_ref[:, cols] = ot.astype(o_ref.dtype)
        cp = pltpu.make_async_copy(o_ref.at[:, cols], o_hbm.at[:, cols], out_sems.at[qb])
        cp.start()
        o_cp.append(cp)

    mq = D // 4
    pieces = [(mi, kt) for mi in range(4) for kt in range(k7 // 128)]
    for qb in range(NQ):
        work = [(u, c) for u in range(HPI) for c in range(nc)]
        otb_scr[...] = ot_scr[qb, 0:k7, :].astype(bf16)
        acc = None
        outs = []
        for i, (mi, kt) in enumerate(pieces):
            rs = slice(mi * mq, (mi + 1) * mq)
            ks = slice(kt * 128, (kt + 1) * 128)
            part = jnp.dot(wot_scr[rs, ks], otb_scr[ks, :], preferred_element_type=f32)
            if kt == 0:
                o3_scr[qb % 2, rs, :] = part
            else:
                o3_scr[qb % 2, rs, :] = o3_scr[qb % 2, rs, :] + part
            if i == 2 and qb > 0:
                finish(qb - 1)
            lo, hi = i * len(work) // len(pieces), (i + 1) * len(work) // len(pieces)
            for (u, c) in work[lo:hi]:
                hh = NH - HPI + u
                buf = u * NQ + qb
                acc = pv_chunk(hh, buf, ms[buf], c, None if c == 0 else acc)
                if c == nc - 1:
                    outs.append(pv_norm(hh, qb, acc))
        pv_store(NH // HPI - 1, qb, outs)
    finish(NQ - 1)
    for cp in o_cp:
        cp.wait()


@jax.jit
def pallas_gated_mix__mha_block__mha_block__prompt_kernel(
    A_x: jax.Array,
    A_wqkv: jax.Array,
    A_wo: jax.Array,
    B_x: jax.Array,
    B_wqkv: jax.Array,
    B_wo: jax.Array,
    gate_w: jax.Array,
):
    xt = A_x.reshape(S, D).T
    out_t = pl.pallas_call(
        _kernel,
        out_shape=jax.ShapeDtypeStruct((D, S), jnp.bfloat16),
        in_specs=[pl.BlockSpec(memory_space=pl.ANY)] * 5 + [pl.BlockSpec(memory_space=pltpu.VMEM)],
        out_specs=pl.BlockSpec(memory_space=pl.ANY),
        scratch_shapes=[
            pltpu.VMEM((NQ, D, TQ), jnp.bfloat16),
            pltpu.VMEM((NB, D, D3), jnp.bfloat16),
            pltpu.VMEM((NB, D, D), jnp.bfloat16),
            pltpu.VMEM((D, S), jnp.bfloat16),
            pltpu.SemaphoreType.DMA((4 + NQ + 2,)),
            pltpu.SemaphoreType.DMA((NQ,)),
            pltpu.VMEM((NB, D3 + GR, D), jnp.bfloat16),
            pltpu.VMEM((D, NB * D), jnp.bfloat16),
            pltpu.VMEM((D3 + GR, TQ), jnp.float32),
            pltpu.VMEM((NG, S, 128), jnp.bfloat16),
            pltpu.VMEM((NG, NQ, 128, TQ), jnp.bfloat16),
            pltpu.VMEM((NH, NQ, DP, TQ), jnp.bfloat16),
            pltpu.VMEM((NB, NQ, 8, TQ), jnp.float32),
            pltpu.VMEM((HPI * NQ, S, TQ), jnp.float32),
            pltpu.VMEM((NQ, NH * DH, TQ), jnp.float32),
            pltpu.VMEM((2, D, TQ), jnp.float32),
            pltpu.VMEM((6 * 128, TQ), jnp.bfloat16),
        ],
        compiler_params=pltpu.CompilerParams(vmem_limit_bytes=100 * 1024 * 1024),
    )(xt, A_wqkv, B_wqkv, A_wo, B_wo, gate_w)
    return out_t.T.reshape(1, S, D)
```
